```python
import jax
import jax.numpy as jnp

def _softmax(x, axis=-1):
    return jax.nn.softmax(x, axis=axis)
def _gelu(x):
    return jax.nn.gelu(x, approximate=True)
def _silu(x):
    return jax.nn.silu(x)
def _sigmoid(x):
    return jax.nn.sigmoid(x)
def _layernorm(x, axis=-1, eps=1e-5):
    m = jnp.mean(x, axis=axis, keepdims=True)
    v = jnp.var(x, axis=axis, keepdims=True)
    return (x - m) / jnp.sqrt(v + eps)
def _scatter_add(tgt, idx, src, axis=0):
    return tgt.at[idx].add(src)
def _segment_sum(src, seg, n):
    return jax.ops.segment_sum(src, seg, n)
class _Rng:
    def __init__(self, key):
        self._k = key
    def _next(self):
        self._k, sub = jax.random.split(self._k)
        return sub
    def normal(self, shape):
        return jax.random.normal(self._next(), shape, dtype=jnp.bfloat16)
    def randint(self, lo, hi, shape):
        return jax.random.randint(self._next(), shape, lo, hi, dtype=jnp.int32)
    def uniform(self, shape, lo=0.0, hi=1.0):
        return jax.random.uniform(self._next(), shape, jnp.bfloat16, lo, hi)
    def permutation(self, n):
        return jax.random.permutation(self._next(), n)


kernel_name = 'interleave_layers__sliding_block__sliding_local_dilated__prompt'

def setup_inputs():
    _rng = _Rng(jax.random.key(int.from_bytes(__import__("os").urandom(4), "little")))
    _w = (lambda a: (lambda t: t.astype(jnp.bfloat16) if jnp.issubdtype(t.dtype, jnp.floating) else t)(jnp.asarray(a)))
    def _A_setup():
        B, S, D = 1, 2048, 1024
        return {
            "x": _w((lambda *s: _rng.normal(s) * 0.05)(B, S, D)),
            "wqkv": _w((lambda *s: _rng.normal(s) * 0.05)(D, 3 * D)),
            "wo": _w((lambda *s: _rng.normal(s) * 0.05)(D, D)),
        }
    _A_in = _A_setup()

    def _B_setup():
        B, S, D = 1, 2048, 1024
        return {
            "x": _w((lambda *s: _rng.normal(s) * 0.05)(B, S, D)),
            "wqkv": _w((lambda *s: _rng.normal(s) * 0.05)(D, 3 * D)),
            "wo": _w((lambda *s: _rng.normal(s) * 0.05)(D, D)),
        }
    _B_in = _B_setup()

    return {
        "A_x": _A_in["x"],
        "A_wqkv": _A_in["wqkv"],
        "A_wo": _A_in["wo"],
        "B_x": _B_in["x"],
        "B_wqkv": _B_in["wqkv"],
        "B_wo": _B_in["wo"],
    }

def reference(A_x, A_wqkv, A_wo, B_x, B_wqkv, B_wo):
    def _A_ref(x, wqkv, wo):
        B, S, D = x.shape
        H = 32; Dh = D // H; W = 256
        qkv = (lambda x, *d: x.transpose(*d))((x @ wqkv).reshape(B, S, 3, H, Dh), 2, 0, 3, 1, 4)
        q, k, v = qkv[0], qkv[1], qkv[2]
        scores = jnp.einsum("bhqd,bhkd->bhqk", q, k) * (Dh ** -0.5)
        idx = jnp.arange(S)
        mask = (idx[:, None] - idx[None, :] >= 0) & (idx[:, None] - idx[None, :] < W)
        scores = jnp.where(mask[None, None], scores, -1e9)
        p = _softmax(scores, axis=-1)
        o = jnp.einsum("bhqk,bhkd->bhqd", p, v)
        return (lambda x, *d: x.transpose(*d))(o, 0, 2, 1, 3).reshape(B, S, D) @ wo

    def _B_ref(x, wqkv, wo):
        B, S, D = x.shape
        H = 32; Dh = D // H
        W, dil = 8, 2
        qkv = (lambda x, *d: x.transpose(*d))((x @ wqkv).reshape(B, S, 3, H, Dh), 2, 0, 3, 1, 4)
        q, k, v = qkv[0], qkv[1], qkv[2]
        scale = Dh ** -0.5
        pos = jnp.arange(S)
        off = jnp.arange(W) * dil
        idx = pos[:, None] - off[None, :]
        mask = idx >= 0
        idx_c = jnp.where(mask, idx, 0).reshape(-1)
        kg = k[:, :, idx_c, :].reshape(B, H, S, W, Dh)
        vg = v[:, :, idx_c, :].reshape(B, H, S, W, Dh)
        logits = jnp.einsum("bhsd,bhswd->bhsw", q, kg) * scale
        logits = jnp.where(mask[None, None, :, :], logits, -1e9)
        attn = _softmax(logits, axis=-1)
        o = jnp.einsum("bhsw,bhswd->bhsd", attn, vg)
        return (lambda x, *d: x.transpose(*d))(o, 0, 2, 1, 3).reshape(B, S, D) @ wo

    x = A_x
    x = x + _A_ref(_layernorm(x, axis=-1), A_wqkv, A_wo)
    x = x + _B_ref(_layernorm(x, axis=-1), B_wqkv, B_wo)
    x = x + _A_ref(_layernorm(x, axis=-1), A_wqkv, A_wo)
    x = x + _B_ref(_layernorm(x, axis=-1), B_wqkv, B_wo)
    return x
```

```python
import functools
import math

import jax
import jax.numpy as jnp
import numpy as np
import jax.experimental.pallas as pl
import jax.experimental.pallas.tpu as pltpu

S = 2048
D = 1024
DH = 32
NG = 8
QC = 128
KT = 32
GR = 16
DM = 256
NEG = -1e30
EPS = 1e-5
QSCALE = (DH ** -0.5) * math.log2(math.e)

WA = 256
WB, DIL = 8, 2
PADB = 16
GS = S + PADB
NU = QC // GR
CFG_A = dict(dmax=WA - 1, step=1, offs=(-16, 0, 16, 240, 256, 272), b0=0)
CFG_B = dict(dmax=(WB - 1) * DIL, step=DIL, offs=(0, 16, 32), b0=6)


def _layernorm(x):
    m = jnp.mean(x, axis=-1, keepdims=True)
    c = x - m
    v = jnp.mean(c * c, axis=-1, keepdims=True)
    return (c * jax.lax.rsqrt(v + EPS)).astype(jnp.bfloat16)


def _recip(x):
    r = pltpu.reciprocal(x, approx=True)
    return r * (2.0 - x * r)


def _ds(start, size):
    if isinstance(start, int):
        return pl.ds(start, size)
    return pl.ds(pl.multiple_of(start, 8), size)


def _ld_bf16(u32_ref, row, n):
    return pltpu.bitcast(u32_ref[_ds(row // 2, n // 2), :], jnp.bfloat16)


def _lane_iota(n):
    return jax.lax.broadcasted_iota(jnp.int32, (n, 128), 1)


def _blockdiag(u32_ref, row, masks):
    u = u32_ref[_ds(row // 2, KT // 2), :]
    return pltpu.bitcast(jnp.concatenate([u & m for m in masks], axis=0), jnp.bfloat16)


def _tiles(cfg, jmin):
    tiles = []
    for j in range(max(jmin, -cfg["dmax"] // KT), QC // KT):
        lo = max(0, (KT * j) // GR)
        hi = min(NU, (KT * j + KT - 1 + cfg["dmax"]) // GR + 1)
        tiles.append((j, lo, hi))
    slots, n = {}, 0
    for j, lo, hi in tiles:
        for u in range(lo, hi):
            slots[u, j] = n
            n += 1
    return tiles, slots


def _seg_reduce(x, seg, red, fill):
    out = None
    for h in range(4):
        r = red(jnp.where(seg == h, x, fill), axis=-1, keepdims=True)
        out = jnp.broadcast_to(r, x.shape) if out is None else jnp.where(seg == h, r, out)
    return out


def _attn(cfg, qu, ku, vu, o_ref, bias_ref, ones_ref, sbufs, mbufs, i0, nchunks, jmin):
    tiles, slots = _tiles(cfg, jmin)
    seg = _lane_iota(GR) // KT

    def masks():
        return [jnp.where(seg == h, jnp.uint32(0xFFFFFFFF), jnp.uint32(0)) for h in range(4)]

    def base(t):
        return (t % NG) * GS + PADB + (t // NG + i0) * QC

    def scores(t, sbuf, mbuf):
        b = base(t)
        um = masks()
        m = [None] * NU
        for j, lo, hi in tiles:
            kbd = _blockdiag(ku, b + KT * j, um)
            q = _ld_bf16(qu, b + GR * lo, GR * (hi - lo))
            res = jax.lax.dot_general(q, kbd, (((1,), (1,)), ((), ())),
                                      preferred_element_type=jnp.float32)
            for u in range(lo, hi):
                x = res[GR * (u - lo):GR * (u - lo + 1)]
                off = GR * u - KT * j
                if off in cfg["offs"]:
                    x = x + bias_ref[cfg["b0"] + cfg["offs"].index(off)]
                sbuf[slots[u, j]] = x
                m[u] = x if m[u] is None else jnp.maximum(m[u], x)
        for u in range(NU):
            mbuf[u] = _seg_reduce(m[u], seg, jnp.max, NEG)

    def softmax_pv(t, sbuf, mbuf):
        b = base(t)
        um = masks()
        p, ls = {}, []
        for u in range(NU):
            m = mbuf[u]
            l = None
            for j, lo, hi in tiles:
                if lo <= u < hi:
                    e = jnp.exp2(sbuf[slots[u, j]] - m)
                    p[u, j] = e
                    l = e if l is None else l + e
            ls.append(l)
        lsum = jnp.dot(jnp.concatenate(ls, axis=0).astype(jnp.bfloat16),
                       pltpu.bitcast(ones_ref[...], jnp.bfloat16),
                       preferred_element_type=jnp.float32)
        linv = _recip(lsum)
        acc = [None] * NU
        for j, lo, hi in tiles:
            vbd = _blockdiag(vu, b + KT * j, um)
            pj = jnp.concatenate([p[u, j] for u in range(lo, hi)], axis=0).astype(jnp.bfloat16)
            res = jnp.dot(pj, vbd, preferred_element_type=jnp.float32)
            for u in range(lo, hi):
                x = res[GR * (u - lo):GR * (u - lo + 1)]
                acc[u] = x if acc[u] is None else acc[u] + x
        o = jnp.concatenate([acc[u] * linv[GR * u:GR * (u + 1)] for u in range(NU)], axis=0)
        orow = (t % NG) * S + (t // NG + i0) * QC
        o_ref[pl.ds(pl.multiple_of(orow, QC), QC), :] = o.astype(jnp.bfloat16)

    n = nchunks * NG
    scores(0, sbufs[0], mbufs[0])

    def body(k, _):
        scores(2 * k + 1, sbufs[1], mbufs[1])
        softmax_pv(2 * k, sbufs[0], mbufs[0])
        scores(jnp.minimum(2 * k + 2, n - 1), sbufs[0], mbufs[0])
        softmax_pv(2 * k + 1, sbufs[1], mbufs[1])
        return 0
    jax.lax.fori_loop(0, n // 2, body, 0)


def _layer_attn(cfg, *a):
    ns = -(-cfg["dmax"] // QC)
    for i in range(ns):
        _attn(cfg, *a, i, 1, -(i * QC) // KT)
    _attn(cfg, *a, ns, S // QC - ns, -10 ** 6)


def _qkv_store(xn, w_ref, q_ref, k_ref, v_ref, r0):
    res = jnp.dot(xn, w_ref[...], preferred_element_type=jnp.float32)
    for n, ref in enumerate((q_ref, k_ref, v_ref)):
        for g in range(NG):
            x = res[:, n * D + g * 128:n * D + (g + 1) * 128]
            if n == 0:
                x = x * QSCALE
            ref[pl.ds(pl.multiple_of(g * GS + PADB + r0, GR), DM), :] = x.astype(jnp.bfloat16)


def _kernel(x_hbm, aq_hbm, ao_hbm, bq_hbm, bo_hbm, out_hbm,
            xin, xres, aq, ao, bq, bo, q_s, k_s, v_s, o_s, s0, s1, m0, m1, bias, ones, sems):
    cps = [pltpu.make_async_copy(src, dst, sems.at[i]) for i, (src, dst) in enumerate(
        [(x_hbm, xin), (aq_hbm, aq), (ao_hbm, ao), (bq_hbm, bq), (bo_hbm, bo)])]
    for c in cps:
        c.start()
    nd = S // DM

    d0 = jax.lax.broadcasted_iota(jnp.int32, (GR, 128), 0) - _lane_iota(GR) % KT
    for cfg in (CFG_A, CFG_B):
        for n, off in enumerate(cfg["offs"]):
            d = d0 + off
            ok = (d >= 0) & (d <= cfg["dmax"]) & (d % cfg["step"] == 0)
            bias[cfg["b0"] + n] = jnp.where(ok, 0.0, NEG).astype(jnp.float32)

    ri = jax.lax.broadcasted_iota(jnp.int32, (64, 128), 0)
    ones[...] = jnp.where((2 * ri) // DH == _lane_iota(64) // DH, jnp.uint32(0x3F803F80), jnp.uint32(0))

    qu, ku, vu, ou = (r.bitcast(jnp.uint32) for r in (q_s, k_s, v_s, o_s))

    def rsl(c):
        return pl.ds(pl.multiple_of(c * DM, DM), DM)

    def attn_out(c, wo):
        o = jnp.concatenate([_ld_bf16(ou, g * S + c * DM, DM) for g in range(NG)], axis=1)
        return xres[rsl(c), :] + jnp.dot(o, wo[...], preferred_element_type=jnp.float32)

    cps[0].wait()
    cps[1].wait()

    def first(c, _):
        x = xin[rsl(c), :].astype(jnp.float32)
        xres[rsl(c), :] = x
        _qkv_store(_layernorm(x), aq, q_s, k_s, v_s, c * DM)
        return 0
    jax.lax.fori_loop(0, nd, first, 0)

    def mid(wo, wq):
        def f(c, _):
            x = attn_out(c, wo)
            xres[rsl(c), :] = x
            _qkv_store(_layernorm(x), wq, q_s, k_s, v_s, c * DM)
            return 0
        jax.lax.fori_loop(0, nd, f, 0)

    def last(c, _):
        xin[rsl(c), :] = attn_out(c, bo).astype(jnp.bfloat16)
        return 0

    def attn_a():
        _layer_attn(CFG_A, qu, ku, vu, o_s, bias, ones, (s0, s1), (m0, m1))

    def attn_b():
        _layer_attn(CFG_B, qu, ku, vu, o_s, bias, ones, (s0, s1), (m0, m1))

    attn_a()
    cps[2].wait()
    cps[3].wait()
    mid(ao, bq)
    attn_b()
    cps[4].wait()
    mid(bo, aq)
    attn_a()
    mid(ao, bq)
    attn_b()
    jax.lax.fori_loop(0, nd, last, 0)
    cp = pltpu.make_async_copy(xin, out_hbm, sems.at[0])
    cp.start()
    cp.wait()


@jax.jit
def pallas_interleave_layers__sliding_block__sliding_local_dilated__prompt_kernel(
    A_x: jax.Array,
    A_wqkv: jax.Array,
    A_wo: jax.Array,
    B_x: jax.Array,
    B_wqkv: jax.Array,
    B_wo: jax.Array,
):
    bf, f32 = jnp.bfloat16, jnp.float32
    NSLOT = len(_tiles(CFG_A, -10 ** 6)[1])
    out = pl.pallas_call(
        _kernel,
        out_shape=jax.ShapeDtypeStruct((S, D), bf),
        in_specs=[pl.BlockSpec(memory_space=pl.ANY)] * 5,
        out_specs=pl.BlockSpec(memory_space=pl.ANY),
        scratch_shapes=[
            pltpu.VMEM((S, D), bf), pltpu.VMEM((S, D), jnp.float32),
            pltpu.VMEM((D, 3 * D), bf), pltpu.VMEM((D, D), bf),
            pltpu.VMEM((D, 3 * D), bf), pltpu.VMEM((D, D), bf),
            pltpu.VMEM((NG * GS, 128), bf), pltpu.VMEM((NG * GS, 128), bf),
            pltpu.VMEM((NG * GS, 128), bf), pltpu.VMEM((NG * S, 128), bf),
            pltpu.VMEM((NSLOT, GR, 128), f32), pltpu.VMEM((NSLOT, GR, 128), f32),
            pltpu.VMEM((NU, GR, 128), f32), pltpu.VMEM((NU, GR, 128), f32),
            pltpu.VMEM((9, GR, 128), f32), pltpu.VMEM((64, 128), jnp.uint32),
            pltpu.SemaphoreType.DMA((5,)),
        ],
        compiler_params=pltpu.CompilerParams(vmem_limit_bytes=100 * 2 ** 20),
    )(A_x.reshape(S, D), A_wqkv, A_wo, B_wqkv, B_wo)
    return out.reshape(1, S, D)
```

```python
import functools
import math

import jax
import jax.numpy as jnp
import numpy as np
import jax.experimental.pallas as pl
import jax.experimental.pallas.tpu as pltpu

S = 2048
D = 1024
DH = 32
NG = 8
QC = 128
KT = 32
GR = 16
DM = 256
NEG = -1e30
EPS = 1e-5
QSCALE = (DH ** -0.5) * math.log2(math.e)

WA = 256
WB, DIL = 8, 2
PADB = 16
GS = S + PADB
NU = QC // GR
CFG_A = dict(dmax=WA - 1, step=1, offs=(-16, 0, 16, 240, 256, 272), b0=0)
CFG_B = dict(dmax=(WB - 1) * DIL, step=DIL, offs=(0, 16, 32), b0=6)


def _layernorm(x):
    m = jnp.mean(x, axis=-1, keepdims=True)
    c = x - m
    v = jnp.mean(c * c, axis=-1, keepdims=True)
    return (c * jax.lax.rsqrt(v + EPS)).astype(jnp.bfloat16)


def _recip(x):
    r = pltpu.reciprocal(x, approx=True)
    return r * (2.0 - x * r)


def _ds(start, size):
    if isinstance(start, int):
        return pl.ds(start, size)
    return pl.ds(pl.multiple_of(start, 8), size)


def _ld_bf16(u32_ref, row, n):
    return pltpu.bitcast(u32_ref[_ds(row // 2, n // 2), :], jnp.bfloat16)


def _lane_iota(n):
    return jax.lax.broadcasted_iota(jnp.int32, (n, 128), 1)


def _blockdiag(u32_ref, row, masks):
    u = u32_ref[_ds(row // 2, KT // 2), :]
    return pltpu.bitcast(jnp.concatenate([u & m for m in masks], axis=0), jnp.bfloat16)


def _tiles(cfg, jmin):
    tiles = []
    for j in range(max(jmin, -cfg["dmax"] // KT), QC // KT):
        lo = max(0, (KT * j) // GR)
        hi = min(NU, (KT * j + KT - 1 + cfg["dmax"]) // GR + 1)
        tiles.append((j, lo, hi))
    slots, n = {}, 0
    for j, lo, hi in tiles:
        for u in range(lo, hi):
            slots[u, j] = n
            n += 1
    return tiles, slots


def _seg_reduce(x, seg, red, fill):
    out = None
    for h in range(4):
        r = red(jnp.where(seg == h, x, fill), axis=-1, keepdims=True)
        out = jnp.broadcast_to(r, x.shape) if out is None else jnp.where(seg == h, r, out)
    return out


def _attn_stages(cfg, qu, ku, vu, o_ref, bias_ref, ones_ref, i0, jmin):
    tiles, slots = _tiles(cfg, jmin)
    seg = _lane_iota(GR) // KT

    def masks():
        return [jnp.where(seg == h, jnp.uint32(0xFFFFFFFF), jnp.uint32(0)) for h in range(4)]

    def base(t):
        return (t % NG) * GS + PADB + (t // NG + i0) * QC

    def scores(t, sbuf, mbuf):
        b = base(t)
        um = masks()
        m = [None] * NU
        for j, lo, hi in tiles:
            kbd = _blockdiag(ku, b + KT * j, um)
            q = _ld_bf16(qu, b + GR * lo, GR * (hi - lo))
            res = jax.lax.dot_general(q, kbd, (((1,), (1,)), ((), ())),
                                      preferred_element_type=jnp.float32)
            for u in range(lo, hi):
                x = res[GR * (u - lo):GR * (u - lo + 1)]
                off = GR * u - KT * j
                if off in cfg["offs"]:
                    x = x + bias_ref[cfg["b0"] + cfg["offs"].index(off)]
                sbuf[slots[u, j]] = x
                m[u] = x if m[u] is None else jnp.maximum(m[u], x)
        for u in range(NU):
            mbuf[u] = _seg_reduce(m[u], seg, jnp.max, NEG)

    def softmax_pv(t, sbuf, mbuf):
        b = base(t)
        um = masks()
        p, ls = {}, []
        for u in range(NU):
            m = mbuf[u]
            l = None
            for j, lo, hi in tiles:
                if lo <= u < hi:
                    e = jnp.exp2(sbuf[slots[u, j]] - m)
                    p[u, j] = e
                    l = e if l is None else l + e
            ls.append(l)
        lsum = jnp.dot(jnp.concatenate(ls, axis=0).astype(jnp.bfloat16),
                       pltpu.bitcast(ones_ref[...], jnp.bfloat16),
                       preferred_element_type=jnp.float32)
        linv = _recip(lsum)
        acc = [None] * NU
        for j, lo, hi in tiles:
            vbd = _blockdiag(vu, b + KT * j, um)
            pj = jnp.concatenate([p[u, j] for u in range(lo, hi)], axis=0).astype(jnp.bfloat16)
            res = jnp.dot(pj, vbd, preferred_element_type=jnp.float32)
            for u in range(lo, hi):
                x = res[GR * (u - lo):GR * (u - lo + 1)]
                acc[u] = x if acc[u] is None else acc[u] + x
        o = jnp.concatenate([acc[u] * linv[GR * u:GR * (u + 1)] for u in range(NU)], axis=0)
        orow = (t % NG) * S + (t // NG + i0) * QC
        o_ref[pl.ds(pl.multiple_of(orow, QC), QC), :] = o.astype(jnp.bfloat16)

    return scores, softmax_pv


def _attn_head(cfg, refs, sbufs, mbufs):
    for i in range(DM // QC):
        scores, softmax_pv = _attn_stages(cfg, *refs, i, -(i * QC) // KT)
        scores(0, sbufs[0], mbufs[0])

        def body(k, _):
            scores(2 * k + 1, sbufs[1], mbufs[1])
            softmax_pv(2 * k, sbufs[0], mbufs[0])
            scores(jnp.minimum(2 * k + 2, NG - 1), sbufs[0], mbufs[0])
            softmax_pv(2 * k + 1, sbufs[1], mbufs[1])
            return 0
        jax.lax.fori_loop(0, NG // 2, body, 0)


PN = 256


def _dense_pieces(c, xres, ou, wo, wq, qkv, final_ref):
    r = pl.ds(pl.multiple_of(c * DM, DM), DM)
    st = {}
    pieces = []

    def proj(n):
        if n == 0:
            st["o"] = jnp.concatenate([_ld_bf16(ou, g * S + c * DM, DM) for g in range(NG)], axis=1)
        cs = pl.ds(n * PN, PN)
        x = xres[r, cs] + jnp.dot(st["o"], wo[:, cs], preferred_element_type=jnp.float32)
        if final_ref is None:
            xres[r, cs] = x
            st["x", n] = x
        else:
            final_ref[r, cs] = x.astype(jnp.bfloat16)

    def qkvp(n):
        if n == 0:
            if wo is None:
                x = st["x0"]
            else:
                x = jnp.concatenate([st["x", k] for k in range(D // PN)], axis=1)
            st["xn"] = _layernorm(x)
        res = jnp.dot(st["xn"], wq[:, pl.ds(n * PN, PN)], preferred_element_type=jnp.float32)
        for k in range(PN // 128):
            col = n * PN + k * 128
            which, g = col // D, (col % D) // 128
            x = res[:, k * 128:(k + 1) * 128]
            if which == 0:
                x = x * QSCALE
            qkv[which][pl.ds(pl.multiple_of(g * GS + PADB + c * DM, GR), DM), :] = x.astype(jnp.bfloat16)

    if wo is not None:
        pieces += [functools.partial(proj, n) for n in range(D // PN)]
    if wq is not None:
        pieces += [functools.partial(qkvp, n) for n in range(3 * D // PN)]
    return st, r, pieces


def _layer(cfg, cur, nxt, o_s, xres, wo, wq, final_ref, consts, sbufs, mbufs):
    refs = tuple(x.bitcast(jnp.uint32) for x in cur) + (o_s,) + consts
    ou = o_s.bitcast(jnp.uint32)
    _attn_head(cfg, refs, sbufs, mbufs)
    scores, softmax_pv = _attn_stages(cfg, *refs, 0, -10 ** 6)
    nstep = (DM // QC) * NG
    nd = S // DM
    tmax = nd * nstep - 1
    scores(nstep, sbufs[0], mbufs[0])

    def body(c, _):
        _, _, pieces = _dense_pieces(c, xres, ou, wo, wq, nxt, final_ref)
        t0 = (c + 1) * nstep
        done = 0
        for s in range(nstep):
            while done < len(pieces) and (done < D // PN or done * nstep <= s * len(pieces)):
                pieces[done]()
                done += 1
            scores(jnp.minimum(t0 + s + 1, tmax), sbufs[(s + 1) % 2], mbufs[(s + 1) % 2])
            softmax_pv(t0 + s, sbufs[s % 2], mbufs[s % 2])
        for pc in pieces[done:]:
            pc()
        return 0
    jax.lax.fori_loop(0, nd - 1, body, 0)
    _, _, pieces = _dense_pieces(nd - 1, xres, ou, wo, wq, nxt, final_ref)
    for pc in pieces:
        pc()


def _kernel(x_hbm, aq_hbm, ao_hbm, bq_hbm, bo_hbm, out_hbm,
            xin, xres, aq, ao, bq, bo, q0, k0, v0, q1, k1, v1, o_s, s0, s1, m0, m1, bias, ones, sems):
    cps = [pltpu.make_async_copy(src, dst, sems.at[i]) for i, (src, dst) in enumerate(
        [(x_hbm, xin), (aq_hbm, aq), (ao_hbm, ao), (bq_hbm, bq), (bo_hbm, bo)])]
    for c in cps:
        c.start()

    d0 = jax.lax.broadcasted_iota(jnp.int32, (GR, 128), 0) - _lane_iota(GR) % KT
    for cfg in (CFG_A, CFG_B):
        for n, off in enumerate(cfg["offs"]):
            d = d0 + off
            ok = (d >= 0) & (d <= cfg["dmax"]) & (d % cfg["step"] == 0)
            bias[cfg["b0"] + n] = jnp.where(ok, 0.0, NEG).astype(jnp.float32)
    ri = jax.lax.broadcasted_iota(jnp.int32, (64, 128), 0)
    ones[...] = jnp.where((2 * ri) // DH == _lane_iota(64) // DH, jnp.uint32(0x3F803F80), jnp.uint32(0))

    cps[0].wait()
    cps[1].wait()
    buf0, buf1 = (q0, k0, v0), (q1, k1, v1)

    def first(c, _):
        st, r, pieces = _dense_pieces(c, xres, None, None, aq, buf0, None)
        st["x0"] = xin[r, :].astype(jnp.float32)
        xres[r, :] = st["x0"]
        for pc in pieces:
            pc()
        return 0
    jax.lax.fori_loop(0, S // DM, first, 0)

    rest = ((bias, ones), (s0, s1), (m0, m1))
    cps[2].wait()
    cps[3].wait()
    _layer(CFG_A, buf0, buf1, o_s, xres, ao, bq, None, *rest)
    cps[4].wait()
    _layer(CFG_B, buf1, buf0, o_s, xres, bo, aq, None, *rest)
    _layer(CFG_A, buf0, buf1, o_s, xres, ao, bq, None, *rest)
    _layer(CFG_B, buf1, buf0, o_s, xres, bo, None, xin, *rest)
    cp = pltpu.make_async_copy(xin, out_hbm, sems.at[0])
    cp.start()
    cp.wait()


@jax.jit
def pallas_interleave_layers__sliding_block__sliding_local_dilated__prompt_kernel(
    A_x: jax.Array,
    A_wqkv: jax.Array,
    A_wo: jax.Array,
    B_x: jax.Array,
    B_wqkv: jax.Array,
    B_wo: jax.Array,
):
    bf, f32 = jnp.bfloat16, jnp.float32
    NSLOT = len(_tiles(CFG_A, -10 ** 6)[1])
    out = pl.pallas_call(
        _kernel,
        out_shape=jax.ShapeDtypeStruct((S, D), bf),
        in_specs=[pl.BlockSpec(memory_space=pl.ANY)] * 5,
        out_specs=pl.BlockSpec(memory_space=pl.ANY),
        scratch_shapes=[
            pltpu.VMEM((S, D), bf), pltpu.VMEM((S, D), jnp.float32),
            pltpu.VMEM((D, 3 * D), bf), pltpu.VMEM((D, D), bf),
            pltpu.VMEM((D, 3 * D), bf), pltpu.VMEM((D, D), bf),
            *[pltpu.VMEM((NG * GS, 128), bf) for _ in range(6)],
            pltpu.VMEM((NG * S, 128), bf),
            pltpu.VMEM((NSLOT, GR, 128), f32), pltpu.VMEM((NSLOT, GR, 128), f32),
            pltpu.VMEM((NU, GR, 128), f32), pltpu.VMEM((NU, GR, 128), f32),
            pltpu.VMEM((9, GR, 128), f32), pltpu.VMEM((64, 128), jnp.uint32),
            pltpu.SemaphoreType.DMA((5,)),
        ],
        compiler_params=pltpu.CompilerParams(vmem_limit_bytes=100 * 2 ** 20),
    )(A_x.reshape(S, D), A_wqkv, A_wo, B_wqkv, B_wo)
    return out.reshape(1, S, D)
```

```python
import functools
import math

import jax
import jax.numpy as jnp
import numpy as np
import jax.experimental.pallas as pl
import jax.experimental.pallas.tpu as pltpu

S = 2048
D = 1024
DH = 32
NG = 8
QC = 128
KT = 32
GR = 16
DM = 256
NEG = -1e30
EPS = 1e-5
QSCALE = (DH ** -0.5) * math.log2(math.e)

WA = 256
WB, DIL = 8, 2
PADB = 16
GS = S + PADB
NU = QC // GR
CFG_A = dict(dmax=WA - 1, step=1, offs=(-16, 0, 16, 240, 256, 272), b0=0)
CFG_B = dict(dmax=(WB - 1) * DIL, step=DIL, offs=(0, 16, 32), b0=6)


def _layernorm(x):
    m = jnp.mean(x, axis=-1, keepdims=True)
    c = x - m
    v = jnp.mean(c * c, axis=-1, keepdims=True)
    return (c * jax.lax.rsqrt(v + EPS)).astype(jnp.bfloat16)


def _recip(x):
    r = pltpu.reciprocal(x, approx=True)
    return r * (2.0 - x * r)


def _ds(start, size):
    if isinstance(start, int):
        return pl.ds(start, size)
    return pl.ds(pl.multiple_of(start, 8), size)


def _ld_bf16(u32_ref, row, n):
    return pltpu.bitcast(u32_ref[_ds(row // 2, n // 2), :], jnp.bfloat16)


def _lane_iota(n):
    return jax.lax.broadcasted_iota(jnp.int32, (n, 128), 1)


def _blockdiag(u32_ref, row, masks):
    u = u32_ref[_ds(row // 2, KT // 2), :]
    return pltpu.bitcast(jnp.concatenate([u & m for m in masks], axis=0), jnp.bfloat16)


def _tiles(cfg, jmin):
    tiles = []
    for j in range(max(jmin, -cfg["dmax"] // KT), QC // KT):
        lo = max(0, (KT * j) // GR)
        hi = min(NU, (KT * j + KT - 1 + cfg["dmax"]) // GR + 1)
        tiles.append((j, lo, hi))
    slots, n = {}, 0
    for j, lo, hi in tiles:
        for u in range(lo, hi):
            slots[u, j] = n
            n += 1
    return tiles, slots


def _seg_reduce(x, seg, red, fill):
    out = None
    for h in range(4):
        r = red(jnp.where(seg == h, x, fill), axis=-1, keepdims=True)
        out = jnp.broadcast_to(r, x.shape) if out is None else jnp.where(seg == h, r, out)
    return out


def _attn_stages(cfg, qu, ku, vu, o_ref, bias_ref, ones_ref, i0, jmin):
    tiles, slots = _tiles(cfg, jmin)
    seg = _lane_iota(GR) // KT

    def masks():
        return [jnp.where(seg == h, jnp.uint32(0xFFFFFFFF), jnp.uint32(0)) for h in range(4)]

    def base(t):
        return (t % NG) * GS + PADB + (t // NG + i0) * QC

    def scores(t, sbuf, mbuf):
        b = base(t)
        um = masks()
        m = [None] * NU
        for j, lo, hi in tiles:
            kbd = _blockdiag(ku, b + KT * j, um)
            q = _ld_bf16(qu, b + GR * lo, GR * (hi - lo))
            res = jax.lax.dot_general(q, kbd, (((1,), (1,)), ((), ())),
                                      preferred_element_type=jnp.float32)
            for u in range(lo, hi):
                x = res[GR * (u - lo):GR * (u - lo + 1)]
                off = GR * u - KT * j
                if off in cfg["offs"]:
                    x = x + bias_ref[cfg["b0"] + cfg["offs"].index(off)]
                sbuf[slots[u, j]] = x
                m[u] = x if m[u] is None else jnp.maximum(m[u], x)
        for u in range(NU):
            mbuf[u] = _seg_reduce(m[u], seg, jnp.max, NEG)

    def softmax_pv(t, sbuf, mbuf):
        b = base(t)
        um = masks()
        p, ls = {}, []
        for u in range(NU):
            m = mbuf[u]
            l = None
            for j, lo, hi in tiles:
                if lo <= u < hi:
                    e = jnp.exp2(sbuf[slots[u, j]] - m)
                    p[u, j] = e
                    l = e if l is None else l + e
            ls.append(l)
        lsum = jnp.dot(jnp.concatenate(ls, axis=0).astype(jnp.bfloat16),
                       pltpu.bitcast(ones_ref[...], jnp.bfloat16),
                       preferred_element_type=jnp.float32)
        linv = _recip(lsum)
        acc = [None] * NU
        for j, lo, hi in tiles:
            vbd = _blockdiag(vu, b + KT * j, um)
            pj = jnp.concatenate([p[u, j] for u in range(lo, hi)], axis=0).astype(jnp.bfloat16)
            res = jnp.dot(pj, vbd, preferred_element_type=jnp.float32)
            for u in range(lo, hi):
                x = res[GR * (u - lo):GR * (u - lo + 1)]
                acc[u] = x if acc[u] is None else acc[u] + x
        o = jnp.concatenate([acc[u] * linv[GR * u:GR * (u + 1)] for u in range(NU)], axis=0)
        orow = (t % NG) * S + (t // NG + i0) * QC
        o_ref[pl.ds(pl.multiple_of(orow, QC), QC), :] = o.astype(jnp.bfloat16)

    return scores, softmax_pv


def _head_steps(cfg, refs, sbufs, mbufs):
    stages = [_attn_stages(cfg, *refs, i, -(i * QC) // KT) for i in range(DM // QC)]
    reg_scores = _attn_stages(cfg, *refs, 0, -10 ** 6)[0]
    n = (DM // QC) * NG

    def step(s):
        if s == 0:
            stages[0][0](0, sbufs[0], mbufs[0])
        nb = (sbufs[(s + 1) % 2], mbufs[(s + 1) % 2])
        if s + 1 < n:
            stages[(s + 1) // NG][0]((s + 1) % NG, *nb)
        else:
            reg_scores(n, *nb)
        stages[s // NG][1](s % NG, sbufs[s % 2], mbufs[s % 2])
    return [functools.partial(step, s) for s in range(n)]


def _interleave(pieces, steps, nfirst):
    done = 0
    for s, st in enumerate(steps):
        while done < len(pieces) and (done < nfirst or done * len(steps) <= s * len(pieces)):
            pieces[done]()
            done += 1
        st()
    for pc in pieces[done:]:
        pc()


PN = 256


def _dense_pieces(c, xres, ou, wo, wq, qkv, final_ref):
    r = pl.ds(pl.multiple_of(c * DM, DM), DM)
    st = {}
    pieces = []

    def proj(n):
        if n == 0:
            st["o"] = jnp.concatenate([_ld_bf16(ou, g * S + c * DM, DM) for g in range(NG)], axis=1)
        cs = pl.ds(n * PN, PN)
        x = xres[r, cs] + jnp.dot(st["o"], wo[:, cs], preferred_element_type=jnp.float32)
        if final_ref is None:
            xres[r, cs] = x
            st["x", n] = x
        else:
            final_ref[r, cs] = x.astype(jnp.bfloat16)

    def qkvp(n):
        if n == 0:
            if wo is None:
                x = st["x0"]
            else:
                x = jnp.concatenate([st["x", k] for k in range(D // PN)], axis=1)
            st["xn"] = _layernorm(x)
        res = jnp.dot(st["xn"], wq[:, pl.ds(n * PN, PN)], preferred_element_type=jnp.float32)
        for k in range(PN // 128):
            col = n * PN + k * 128
            which, g = col // D, (col % D) // 128
            x = res[:, k * 128:(k + 1) * 128]
            if which == 0:
                x = x * QSCALE
            qkv[which][pl.ds(pl.multiple_of(g * GS + PADB + c * DM, GR), DM), :] = x.astype(jnp.bfloat16)

    if wo is not None:
        pieces += [functools.partial(proj, n) for n in range(D // PN)]
    if wq is not None:
        pieces += [functools.partial(qkvp, n) for n in range(3 * D // PN)]
    return st, r, pieces


def _layer(cfg, cur, nxt, o_s, xres, wo, wq, final_ref, consts, sbufs, mbufs, next_head, after_chunk):
    refs = tuple(x.bitcast(jnp.uint32) for x in cur) + (o_s,) + consts
    ou = o_s.bitcast(jnp.uint32)
    scores, softmax_pv = _attn_stages(cfg, *refs, 0, -10 ** 6)
    nstep = (DM // QC) * NG
    nd = S // DM
    tmax = nd * nstep - 1

    def body(c, _):
        _, _, pieces = _dense_pieces(c, xres, ou, wo, wq, nxt, final_ref)
        t0 = (c + 1) * nstep

        def step(s):
            scores(jnp.minimum(t0 + s + 1, tmax), sbufs[(s + 1) % 2], mbufs[(s + 1) % 2])
            softmax_pv(t0 + s, sbufs[s % 2], mbufs[s % 2])
        _interleave(pieces, [functools.partial(step, s) for s in range(nstep)], D // PN)
        after_chunk(c)
        return 0
    jax.lax.fori_loop(0, nd - 1, body, 0)
    _, _, pieces = _dense_pieces(nd - 1, xres, ou, wo, wq, nxt, final_ref)
    _interleave(pieces, next_head, D // PN)
    after_chunk(nd - 1)


def _kernel(x_hbm, aq_hbm, ao_hbm, bq_hbm, bo_hbm, out_hbm,
            xin, xres, aq, ao, bq, bo, q0, k0, v0, q1, k1, v1, o_s, s0, s1, m0, m1, bias, ones,
            sems, xsems, wsems):
    nd = S // DM
    npc = 3 * D // PN

    def rows(c):
        return pl.ds(pl.multiple_of(c * DM, DM), DM)

    def x_copy(c):
        return pltpu.make_async_copy(x_hbm.at[rows(c)], xin.at[rows(c)], xsems.at[c])

    def out_copy(c):
        return pltpu.make_async_copy(xin.at[rows(c)], out_hbm.at[rows(c)], xsems.at[c])

    aq_copies = [pltpu.make_async_copy(aq_hbm.at[:, pl.ds(n * PN, PN)], aq.at[:, pl.ds(n * PN, PN)],
                                       wsems.at[n]) for n in range(npc)]
    cps = [pltpu.make_async_copy(src, dst, sems.at[i]) for i, (src, dst) in enumerate(
        [(ao_hbm, ao), (bq_hbm, bq), (bo_hbm, bo)])]
    x_copy(0).start()
    for c in aq_copies:
        c.start()
    for c in range(1, nd):
        x_copy(c).start()
    for c in cps:
        c.start()

    d0 = jax.lax.broadcasted_iota(jnp.int32, (GR, 128), 0) - _lane_iota(GR) % KT
    for cfg in (CFG_A, CFG_B):
        for n, off in enumerate(cfg["offs"]):
            d = d0 + off
            ok = (d >= 0) & (d <= cfg["dmax"]) & (d % cfg["step"] == 0)
            bias[cfg["b0"] + n] = jnp.where(ok, 0.0, NEG).astype(jnp.float32)
    ri = jax.lax.broadcasted_iota(jnp.int32, (64, 128), 0)
    ones[...] = jnp.where((2 * ri) // DH == _lane_iota(64) // DH, jnp.uint32(0x3F803F80), jnp.uint32(0))

    buf0, buf1 = (q0, k0, v0), (q1, k1, v1)
    consts, sbufs, mbufs = (bias, ones), (s0, s1), (m0, m1)

    def head(cfg, cur):
        refs = tuple(x.bitcast(jnp.uint32) for x in cur) + (o_s,) + consts
        return _head_steps(cfg, refs, sbufs, mbufs)

    def first(c, steps=(), waits=None):
        x_copy(c).wait()
        st, r, pieces = _dense_pieces(c, xres, None, None, aq, buf0, None)
        st["x0"] = xin[r, :].astype(jnp.float32)
        xres[r, :] = st["x0"]
        if waits is not None:
            pieces = [functools.partial(lambda w, p: (w.wait(), p()), w, p) for w, p in zip(waits, pieces)]
        _interleave(pieces, steps, 0)

    first(0, waits=aq_copies)
    jax.lax.fori_loop(1, nd - 1, lambda c, _: first(c), None)
    first(nd - 1, head(CFG_A, buf0))

    def nothing(c):
        pass

    cps[0].wait()
    cps[1].wait()
    _layer(CFG_A, buf0, buf1, o_s, xres, ao, bq, None, consts, sbufs, mbufs, head(CFG_B, buf1), nothing)
    cps[2].wait()
    _layer(CFG_B, buf1, buf0, o_s, xres, bo, aq, None, consts, sbufs, mbufs, head(CFG_A, buf0), nothing)
    _layer(CFG_A, buf0, buf1, o_s, xres, ao, bq, None, consts, sbufs, mbufs, head(CFG_B, buf1), nothing)
    _layer(CFG_B, buf1, buf0, o_s, xres, bo, None, xin, consts, sbufs, mbufs, (),
           lambda c: out_copy(c).start())
    for c in range(nd):
        out_copy(c).wait()


@jax.jit
def pallas_interleave_layers__sliding_block__sliding_local_dilated__prompt_kernel(
    A_x: jax.Array,
    A_wqkv: jax.Array,
    A_wo: jax.Array,
    B_x: jax.Array,
    B_wqkv: jax.Array,
    B_wo: jax.Array,
):
    bf, f32 = jnp.bfloat16, jnp.float32
    NSLOT = len(_tiles(CFG_A, -10 ** 6)[1])
    out = pl.pallas_call(
        _kernel,
        out_shape=jax.ShapeDtypeStruct((S, D), bf),
        in_specs=[pl.BlockSpec(memory_space=pl.ANY)] * 5,
        out_specs=pl.BlockSpec(memory_space=pl.ANY),
        scratch_shapes=[
            pltpu.VMEM((S, D), bf), pltpu.VMEM((S, D), jnp.float32),
            pltpu.VMEM((D, 3 * D), bf), pltpu.VMEM((D, D), bf),
            pltpu.VMEM((D, 3 * D), bf), pltpu.VMEM((D, D), bf),
            *[pltpu.VMEM((NG * GS, 128), bf) for _ in range(6)],
            pltpu.VMEM((NG * S, 128), bf),
            pltpu.VMEM((NSLOT, GR, 128), f32), pltpu.VMEM((NSLOT, GR, 128), f32),
            pltpu.VMEM((NU, GR, 128), f32), pltpu.VMEM((NU, GR, 128), f32),
            pltpu.VMEM((9, GR, 128), f32), pltpu.VMEM((64, 128), jnp.uint32),
            pltpu.SemaphoreType.DMA((3,)), pltpu.SemaphoreType.DMA((S // DM,)),
            pltpu.SemaphoreType.DMA((3 * D // PN,)),
        ],
        compiler_params=pltpu.CompilerParams(vmem_limit_bytes=100 * 2 ** 20),
    )(A_x.reshape(S, D), A_wqkv, A_wo, B_wqkv, B_wo)
    return out.reshape(1, S, D)
```

```python
import functools
import math

import jax
import jax.numpy as jnp
import numpy as np
import jax.experimental.pallas as pl
import jax.experimental.pallas.tpu as pltpu

S = 2048
D = 1024
DH = 32
NG = 8
QC = 128
KT = 32
GR = 16
DM = 256
NEG = -1e30
EPS = 1e-5
QSCALE = (DH ** -0.5) * math.log2(math.e)

WA = 256
WB, DIL = 8, 2
PADB = 16
GS = S + PADB
NU = QC // GR
CFG_A = dict(dmax=WA - 1, step=1, offs=(-16, 0, 16, 240, 256, 272), b0=0)
CFG_B = dict(dmax=(WB - 1) * DIL, step=DIL, offs=(0, 16, 32), b0=6)


def _layernorm(x):
    m = jnp.mean(x, axis=-1, keepdims=True)
    c = x - m
    v = jnp.mean(c * c, axis=-1, keepdims=True)
    return (c * jax.lax.rsqrt(v + EPS)).astype(jnp.bfloat16)


def _recip(x):
    r = pltpu.reciprocal(x, approx=True)
    return r * (2.0 - x * r)


def _ds(start, size):
    if isinstance(start, int):
        return pl.ds(start, size)
    return pl.ds(pl.multiple_of(start, 8), size)


def _ld_bf16(u32_ref, row, n):
    return pltpu.bitcast(u32_ref[_ds(row // 2, n // 2), :], jnp.bfloat16)


def _lane_iota(n):
    return jax.lax.broadcasted_iota(jnp.int32, (n, 128), 1)


def _blockdiag(u32_ref, row, masks):
    u = u32_ref[_ds(row // 2, KT // 2), :]
    return pltpu.bitcast(jnp.concatenate([u & m for m in masks], axis=0), jnp.bfloat16)


def _tiles(cfg, jmin):
    tiles = []
    for j in range(max(jmin, -cfg["dmax"] // KT), QC // KT):
        lo = max(0, (KT * j) // GR)
        hi = min(NU, (KT * j + KT - 1 + cfg["dmax"]) // GR + 1)
        tiles.append((j, lo, hi))
    slots, n = {}, 0
    for j, lo, hi in tiles:
        for u in range(lo, hi):
            slots[u, j] = n
            n += 1
    return tiles, slots


def _seg_reduce(x, seg, red, fill):
    out = None
    for h in range(4):
        r = red(jnp.where(seg == h, x, fill), axis=-1, keepdims=True)
        out = jnp.broadcast_to(r, x.shape) if out is None else jnp.where(seg == h, r, out)
    return out


def _attn_stages(cfg, qu, ku, vu, o_ref, bias_ref, ones_ref, i0, jmin):
    tiles, slots = _tiles(cfg, jmin)
    seg = _lane_iota(GR) // KT

    def masks():
        return [jnp.where(seg == h, jnp.uint32(0xFFFFFFFF), jnp.uint32(0)) for h in range(4)]

    def base(t):
        return (t % NG) * GS + PADB + (t // NG + i0) * QC

    def scores(t, sbuf, mbuf):
        b = base(t)
        um = masks()
        m = [None] * NU
        for j, lo, hi in tiles:
            kbd = _blockdiag(ku, b + KT * j, um)
            q = _ld_bf16(qu, b + GR * lo, GR * (hi - lo))
            res = jax.lax.dot_general(q, kbd, (((1,), (1,)), ((), ())),
                                      preferred_element_type=jnp.float32)
            for u in range(lo, hi):
                x = res[GR * (u - lo):GR * (u - lo + 1)]
                off = GR * u - KT * j
                if off in cfg["offs"]:
                    x = x + bias_ref[cfg["b0"] + cfg["offs"].index(off)]
                sbuf[slots[u, j]] = x
                m[u] = x if m[u] is None else jnp.maximum(m[u], x)
        for u in range(NU):
            mbuf[u] = _seg_reduce(m[u], seg, jnp.max, NEG)

    def softmax_pv(t, sbuf, mbuf):
        b = base(t)
        um = masks()
        p, ls = {}, []
        for u in range(NU):
            m = mbuf[u]
            l = None
            for j, lo, hi in tiles:
                if lo <= u < hi:
                    e = jnp.exp2(sbuf[slots[u, j]] - m)
                    p[u, j] = e
                    l = e if l is None else l + e
            ls.append(l)
        lsum = jnp.dot(jnp.concatenate(ls, axis=0).astype(jnp.bfloat16),
                       pltpu.bitcast(ones_ref[...], jnp.bfloat16),
                       preferred_element_type=jnp.float32)
        if cfg['step'] == 1:
            lsum = jnp.concatenate([_seg_reduce(l, seg, jnp.sum, 0.0) for l in ls], axis=0)
        linv = _recip(lsum)
        acc = [None] * NU
        for j, lo, hi in tiles:
            vbd = _blockdiag(vu, b + KT * j, um)
            pj = jnp.concatenate([p[u, j] for u in range(lo, hi)], axis=0).astype(jnp.bfloat16)
            res = jnp.dot(pj, vbd, preferred_element_type=jnp.float32)
            for u in range(lo, hi):
                x = res[GR * (u - lo):GR * (u - lo + 1)]
                acc[u] = x if acc[u] is None else acc[u] + x
        o = jnp.concatenate([acc[u] * linv[GR * u:GR * (u + 1)] for u in range(NU)], axis=0)
        orow = (t % NG) * S + (t // NG + i0) * QC
        o_ref[pl.ds(pl.multiple_of(orow, QC), QC), :] = o.astype(jnp.bfloat16)

    return scores, softmax_pv


def _head_steps(cfg, refs, sbufs, mbufs):
    stages = [_attn_stages(cfg, *refs, i, -(i * QC) // KT) for i in range(DM // QC)]
    reg_scores = _attn_stages(cfg, *refs, 0, -10 ** 6)[0]
    n = (DM // QC) * NG

    def step(s):
        if s == 0:
            stages[0][0](0, sbufs[0], mbufs[0])
        nb = (sbufs[(s + 1) % 2], mbufs[(s + 1) % 2])
        if s + 1 < n:
            stages[(s + 1) // NG][0]((s + 1) % NG, *nb)
        else:
            reg_scores(n, *nb)
        stages[s // NG][1](s % NG, sbufs[s % 2], mbufs[s % 2])
    return [functools.partial(step, s) for s in range(n)]


def _interleave(pieces, steps, nfirst):
    done = 0
    for s, st in enumerate(steps):
        while done < len(pieces) and (done < nfirst or done * len(steps) <= s * len(pieces)):
            pieces[done]()
            done += 1
        st()
    for pc in pieces[done:]:
        pc()


PN = 256


def _dense_pieces(c, xres, ou, wo, wq, qkv, final_ref):
    r = pl.ds(pl.multiple_of(c * DM, DM), DM)
    st = {}
    pieces = []

    def proj(n):
        if n == 0:
            st["o"] = jnp.concatenate([_ld_bf16(ou, g * S + c * DM, DM) for g in range(NG)], axis=1)
        cs = pl.ds(n * PN, PN)
        x = xres[r, cs] + jnp.dot(st["o"], wo[:, cs], preferred_element_type=jnp.float32)
        if final_ref is None:
            xres[r, cs] = x
            st["x", n] = x
        else:
            final_ref[r, cs] = x.astype(jnp.bfloat16)

    def qkvp(n):
        if n == 0:
            if wo is None:
                x = st["x0"]
            else:
                x = jnp.concatenate([st["x", k] for k in range(D // PN)], axis=1)
            st["xn"] = _layernorm(x)
        res = jnp.dot(st["xn"], wq[:, pl.ds(n * PN, PN)], preferred_element_type=jnp.float32)
        for k in range(PN // 128):
            col = n * PN + k * 128
            which, g = col // D, (col % D) // 128
            x = res[:, k * 128:(k + 1) * 128]
            if which == 0:
                x = x * QSCALE
            qkv[which][pl.ds(pl.multiple_of(g * GS + PADB + c * DM, GR), DM), :] = x.astype(jnp.bfloat16)

    if wo is not None:
        pieces += [functools.partial(proj, n) for n in range(D // PN)]
    if wq is not None:
        pieces += [functools.partial(qkvp, n) for n in range(3 * D // PN)]
    return st, r, pieces


def _layer(cfg, cur, nxt, o_s, xres, wo, wq, final_ref, consts, sbufs, mbufs, next_head, after_chunk):
    refs = tuple(x.bitcast(jnp.uint32) for x in cur) + (o_s,) + consts
    ou = o_s.bitcast(jnp.uint32)
    scores, softmax_pv = _attn_stages(cfg, *refs, 0, -10 ** 6)
    nstep = (DM // QC) * NG
    nd = S // DM
    tmax = nd * nstep - 1

    def body(c, _):
        _, _, pieces = _dense_pieces(c, xres, ou, wo, wq, nxt, final_ref)
        t0 = (c + 1) * nstep

        def step(s):
            scores(jnp.minimum(t0 + s + 1, tmax), sbufs[(s + 1) % 2], mbufs[(s + 1) % 2])
            softmax_pv(t0 + s, sbufs[s % 2], mbufs[s % 2])
        _interleave(pieces, [functools.partial(step, s) for s in range(nstep)], 1)
        after_chunk(c)
        return 0
    jax.lax.fori_loop(0, nd - 1, body, 0)
    _, _, pieces = _dense_pieces(nd - 1, xres, ou, wo, wq, nxt, final_ref)
    _interleave(pieces, next_head, 1)
    after_chunk(nd - 1)


def _kernel(x_hbm, aq_hbm, ao_hbm, bq_hbm, bo_hbm, out_hbm,
            xin, xres, aq, ao, bq, bo, q0, k0, v0, q1, k1, v1, o_s, s0, s1, m0, m1, bias, ones,
            sems, xsems, wsems):
    nd = S // DM
    npc = 3 * D // PN

    def rows(c):
        return pl.ds(pl.multiple_of(c * DM, DM), DM)

    def x_copy(c):
        return pltpu.make_async_copy(x_hbm.at[rows(c)], xin.at[rows(c)], xsems.at[c])

    def out_copy(c):
        return pltpu.make_async_copy(xin.at[rows(c)], out_hbm.at[rows(c)], xsems.at[c])

    aq_copies = [pltpu.make_async_copy(aq_hbm.at[:, pl.ds(n * PN, PN)], aq.at[:, pl.ds(n * PN, PN)],
                                       wsems.at[n]) for n in range(npc)]
    cps = [pltpu.make_async_copy(src, dst, sems.at[i]) for i, (src, dst) in enumerate(
        [(ao_hbm, ao), (bq_hbm, bq), (bo_hbm, bo)])]
    x_copy(0).start()
    for c in aq_copies:
        c.start()
    for c in range(1, nd):
        x_copy(c).start()
    for c in cps:
        c.start()

    d0 = jax.lax.broadcasted_iota(jnp.int32, (GR, 128), 0) - _lane_iota(GR) % KT
    for cfg in (CFG_A, CFG_B):
        for n, off in enumerate(cfg["offs"]):
            d = d0 + off
            ok = (d >= 0) & (d <= cfg["dmax"]) & (d % cfg["step"] == 0)
            bias[cfg["b0"] + n] = jnp.where(ok, 0.0, NEG).astype(jnp.float32)
    ri = jax.lax.broadcasted_iota(jnp.int32, (64, 128), 0)
    ones[...] = jnp.where((2 * ri) // DH == _lane_iota(64) // DH, jnp.uint32(0x3F803F80), jnp.uint32(0))

    buf0, buf1 = (q0, k0, v0), (q1, k1, v1)
    consts, sbufs, mbufs = (bias, ones), (s0, s1), (m0, m1)

    def head(cfg, cur):
        refs = tuple(x.bitcast(jnp.uint32) for x in cur) + (o_s,) + consts
        return _head_steps(cfg, refs, sbufs, mbufs)

    def first(c, steps=(), waits=None):
        x_copy(c).wait()
        st, r, pieces = _dense_pieces(c, xres, None, None, aq, buf0, None)
        st["x0"] = xin[r, :].astype(jnp.float32)
        xres[r, :] = st["x0"]
        if waits is not None:
            pieces = [functools.partial(lambda w, p: (w.wait(), p()), w, p) for w, p in zip(waits, pieces)]
        _interleave(pieces, steps, 0)

    first(0, waits=aq_copies)
    jax.lax.fori_loop(1, nd - 1, lambda c, _: first(c), None)
    first(nd - 1, head(CFG_A, buf0))

    def nothing(c):
        pass

    cps[0].wait()
    cps[1].wait()
    _layer(CFG_A, buf0, buf1, o_s, xres, ao, bq, None, consts, sbufs, mbufs, head(CFG_B, buf1), nothing)
    cps[2].wait()
    _layer(CFG_B, buf1, buf0, o_s, xres, bo, aq, None, consts, sbufs, mbufs, head(CFG_A, buf0), nothing)
    _layer(CFG_A, buf0, buf1, o_s, xres, ao, bq, None, consts, sbufs, mbufs, head(CFG_B, buf1), nothing)
    _layer(CFG_B, buf1, buf0, o_s, xres, bo, None, xin, consts, sbufs, mbufs, (),
           lambda c: out_copy(c).start())
    for c in range(nd):
        out_copy(c).wait()


@jax.jit
def pallas_interleave_layers__sliding_block__sliding_local_dilated__prompt_kernel(
    A_x: jax.Array,
    A_wqkv: jax.Array,
    A_wo: jax.Array,
    B_x: jax.Array,
    B_wqkv: jax.Array,
    B_wo: jax.Array,
):
    bf, f32 = jnp.bfloat16, jnp.float32
    NSLOT = len(_tiles(CFG_A, -10 ** 6)[1])
    out = pl.pallas_call(
        _kernel,
        out_shape=jax.ShapeDtypeStruct((S, D), bf),
        in_specs=[pl.BlockSpec(memory_space=pl.ANY)] * 5,
        out_specs=pl.BlockSpec(memory_space=pl.ANY),
        scratch_shapes=[
            pltpu.VMEM((S, D), bf), pltpu.VMEM((S, D), jnp.float32),
            pltpu.VMEM((D, 3 * D), bf), pltpu.VMEM((D, D), bf),
            pltpu.VMEM((D, 3 * D), bf), pltpu.VMEM((D, D), bf),
            *[pltpu.VMEM((NG * GS, 128), bf) for _ in range(6)],
            pltpu.VMEM((NG * S, 128), bf),
            pltpu.VMEM((NSLOT, GR, 128), f32), pltpu.VMEM((NSLOT, GR, 128), f32),
            pltpu.VMEM((NU, GR, 128), f32), pltpu.VMEM((NU, GR, 128), f32),
            pltpu.VMEM((9, GR, 128), f32), pltpu.VMEM((64, 128), jnp.uint32),
            pltpu.SemaphoreType.DMA((3,)), pltpu.SemaphoreType.DMA((S // DM,)),
            pltpu.SemaphoreType.DMA((3 * D // PN,)),
        ],
        compiler_params=pltpu.CompilerParams(vmem_limit_bytes=100 * 2 ** 20),
    )(A_x.reshape(S, D), A_wqkv, A_wo, B_wqkv, B_wo)
    return out.reshape(1, S, D)
```

```python
import functools
import math

import jax
import jax.numpy as jnp
import numpy as np
import jax.experimental.pallas as pl
import jax.experimental.pallas.tpu as pltpu

S = 2048
D = 1024
DH = 32
NG = 8
QC = 128
KT = 32
GR = 16
DM = 256
NEG = -1e30
EPS = 1e-5
QSCALE = (DH ** -0.5) * math.log2(math.e)

WA = 256
WB, DIL = 8, 2
PADB = 16
GS = S + PADB
NU = QC // GR
CFG_A = dict(dmax=WA - 1, step=1, offs=(-16, 0, 16, 240, 256, 272), b0=0)
CFG_B = dict(dmax=(WB - 1) * DIL, step=DIL, offs=(0, 16, 32), b0=6)


def _layernorm(x):
    m = jnp.mean(x, axis=-1, keepdims=True)
    c = x - m
    v = jnp.mean(c * c, axis=-1, keepdims=True)
    return c * jax.lax.rsqrt(v + EPS)


def _recip(x):
    r = pltpu.reciprocal(x, approx=True)
    return r * (2.0 - x * r)


def _ds(start, size):
    if isinstance(start, int):
        return pl.ds(start, size)
    return pl.ds(pl.multiple_of(start, 8), size)


def _ld_bf16(u32_ref, row, n):
    return pltpu.bitcast(u32_ref[_ds(row // 2, n // 2), :], jnp.bfloat16)


def _lane_iota(n):
    return jax.lax.broadcasted_iota(jnp.int32, (n, 128), 1)


def _blockdiag(u32_ref, row, masks):
    u = u32_ref[_ds(row // 2, KT // 2), :]
    return pltpu.bitcast(jnp.concatenate([u & m for m in masks], axis=0), jnp.bfloat16)


def _tiles(cfg, jmin):
    tiles = []
    for j in range(max(jmin, -cfg["dmax"] // KT), QC // KT):
        lo = max(0, (KT * j) // GR)
        hi = min(NU, (KT * j + KT - 1 + cfg["dmax"]) // GR + 1)
        tiles.append((j, lo, hi))
    slots, n = {}, 0
    for j, lo, hi in tiles:
        for u in range(lo, hi):
            slots[u, j] = n
            n += 1
    return tiles, slots


def _seg_reduce(x, seg, red, fill):
    out = None
    for h in range(4):
        r = red(jnp.where(seg == h, x, fill), axis=-1, keepdims=True)
        out = jnp.broadcast_to(r, x.shape) if out is None else jnp.where(seg == h, r, out)
    return out


def _attn_stages(cfg, qu, ku, vu, o_ref, bias_ref, ones_ref, i0, jmin):
    tiles, slots = _tiles(cfg, jmin)
    seg = _lane_iota(GR) // KT

    def masks():
        return [jnp.where(seg == h, jnp.uint32(0xFFFFFFFF), jnp.uint32(0)) for h in range(4)]

    def base(t):
        return (t % NG) * GS + PADB + (t // NG + i0) * QC

    def scores(t, sbuf, mbuf):
        b = base(t)
        um = masks()
        m = [None] * NU
        for j, lo, hi in tiles:
            kbd = _blockdiag(ku, b + KT * j, um)
            q = _ld_bf16(qu, b + GR * lo, GR * (hi - lo))
            res = jax.lax.dot_general(q, kbd, (((1,), (1,)), ((), ())),
                                      preferred_element_type=jnp.float32)
            for u in range(lo, hi):
                x = res[GR * (u - lo):GR * (u - lo + 1)]
                off = GR * u - KT * j
                if off in cfg["offs"]:
                    x = x + bias_ref[cfg["b0"] + cfg["offs"].index(off)]
                sbuf[slots[u, j]] = x
                m[u] = x if m[u] is None else jnp.maximum(m[u], x)
        for u in range(NU):
            mbuf[u] = _seg_reduce(m[u], seg, jnp.max, NEG)

    def softmax_pv(t, sbuf, mbuf):
        b = base(t)
        um = masks()
        p, ls = {}, []
        for u in range(NU):
            m = mbuf[u]
            l = None
            for j, lo, hi in tiles:
                if lo <= u < hi:
                    e = jnp.exp2(sbuf[slots[u, j]] - m)
                    p[u, j] = e
                    l = e if l is None else l + e
            ls.append(l)
        lsum = jnp.dot(jnp.concatenate(ls, axis=0).astype(jnp.bfloat16),
                       pltpu.bitcast(ones_ref[...], jnp.bfloat16),
                       preferred_element_type=jnp.float32)
        if cfg['step'] == 1:
            lsum = jnp.concatenate([_seg_reduce(l, seg, jnp.sum, 0.0) for l in ls], axis=0)
        linv = _recip(lsum)
        acc = [None] * NU
        for j, lo, hi in tiles:
            vbd = _blockdiag(vu, b + KT * j, um)
            pj = jnp.concatenate([p[u, j] for u in range(lo, hi)], axis=0).astype(jnp.bfloat16)
            res = jnp.dot(pj, vbd, preferred_element_type=jnp.float32)
            for u in range(lo, hi):
                x = res[GR * (u - lo):GR * (u - lo + 1)]
                acc[u] = x if acc[u] is None else acc[u] + x
        o = jnp.concatenate([acc[u] * linv[GR * u:GR * (u + 1)] for u in range(NU)], axis=0)
        orow = (t % NG) * S + (t // NG + i0) * QC
        o_ref[pl.ds(pl.multiple_of(orow, QC), QC), :] = o.astype(jnp.bfloat16)

    return scores, softmax_pv


def _head_steps(cfg, refs, sbufs, mbufs):
    stages = [_attn_stages(cfg, *refs, i, -(i * QC) // KT) for i in range(DM // QC)]
    reg_scores = _attn_stages(cfg, *refs, 0, -10 ** 6)[0]
    n = (DM // QC) * NG

    def step(s):
        if s == 0:
            stages[0][0](0, sbufs[0], mbufs[0])
        nb = (sbufs[(s + 1) % 2], mbufs[(s + 1) % 2])
        if s + 1 < n:
            stages[(s + 1) // NG][0]((s + 1) % NG, *nb)
        else:
            reg_scores(n, *nb)
        stages[s // NG][1](s % NG, sbufs[s % 2], mbufs[s % 2])
    return [functools.partial(step, s) for s in range(n)]


def _interleave(pieces, steps, nfirst):
    done = 0
    for s, st in enumerate(steps):
        while done < len(pieces) and (done < nfirst or done * len(steps) <= s * len(pieces)):
            pieces[done]()
            done += 1
        st()
    for pc in pieces[done:]:
        pc()


PN = 256
HM, HK = DM // 2, D // 2
f32, bf16 = jnp.float32, jnp.bfloat16


def _prep_weights(w, ws, n):
    hn = w.shape[1] // 2
    ca, cb = pl.ds(pl.multiple_of(n * PN, PN), PN), pl.ds(pl.multiple_of(hn + n * PN, PN), PN)
    b11, b12 = w[:HK, ca].astype(f32), w[:HK, cb].astype(f32)
    b21, b22 = w[HK:, ca].astype(f32), w[HK:, cb].astype(f32)
    for i, v in enumerate((b11 + b22, b12 - b22, b21 - b11, b11 + b12, b21 + b22)):
        ws[i, :, ca] = v.astype(bf16)


def _strassen(get_a, w, ws, emit):
    hn = w.shape[1] // 2
    st = {}

    def lhs():
        a = get_a()
        a11, a12, a21, a22 = a[:HM, :HK], a[:HM, HK:], a[HM:, :HK], a[HM:, HK:]
        st["a"] = [v.astype(bf16) for v in
                   (a11 + a22, a21 + a22, a11, a22, a11 + a12, a21 - a11, a12 - a22)]

    def mm(i, n):
        ca, cb = pl.ds(n * PN, PN), pl.ds(hn + n * PN, PN)
        rhs = (lambda: ws[0, :, ca], lambda: w[:HK, ca], lambda: ws[1, :, ca], lambda: ws[2, :, ca],
               lambda: w[HK:, cb], lambda: ws[3, :, ca], lambda: ws[4, :, ca])[i - 1]()
        return jnp.dot(st["a"][i - 1], rhs, preferred_element_type=f32)

    def p1(n):
        if n == 0:
            lhs()
        st["m"] = (mm(1, n), mm(4, n), mm(3, n))

    def p2(n):
        m1, m4, m3 = st["m"]
        m5 = mm(5, n)
        emit(0, hn + n * PN, m3 + m5)
        emit(0, n * PN, m1 + m4 - m5 + mm(7, n))

    def p3(n):
        m1, m4, m3 = st["m"]
        m2 = mm(2, n)
        emit(HM, n * PN, m2 + m4)
        emit(HM, hn + n * PN, m1 - m2 + m3 + mm(6, n))

    return [functools.partial(p, n) for n in range(hn // PN) for p in (p1, p2, p3)]


def _dense_pieces(c, xres, ou, wo, wq, qkv, final_ref):
    r = pl.ds(pl.multiple_of(c * DM, DM), DM)
    st = {}
    pieces = []

    def rws(r0):
        return pl.ds(pl.multiple_of(c * DM + r0, HM), HM)

    def get_o():
        return jnp.concatenate([_ld_bf16(ou, g * S + c * DM, DM) for g in range(NG)], axis=1).astype(f32)

    def emit_x(r0, c0, y):
        x = xres[rws(r0), pl.ds(c0, PN)] + y
        if final_ref is None:
            xres[rws(r0), pl.ds(c0, PN)] = x
            st["x", r0, c0] = x
        else:
            final_ref[rws(r0), pl.ds(c0, PN)] = x.astype(bf16)

    def get_xn():
        if wo is None:
            x = st["x0"]
        else:
            x = jnp.concatenate([jnp.concatenate([st["x", r0, c0] for c0 in range(0, D, PN)], axis=1)
                                 for r0 in (0, HM)], axis=0)
        return _layernorm(x)

    def emit_qkv(r0, c0, res):
        for k in range(PN // 128):
            col = c0 + k * 128
            which, g = col // D, (col % D) // 128
            x = res[:, k * 128:(k + 1) * 128]
            if which == 0:
                x = x * QSCALE
            qkv[which][pl.ds(pl.multiple_of(g * GS + PADB + c * DM + r0, GR), HM), :] = x.astype(bf16)

    if wo is not None:
        pieces += _strassen(get_o, *wo, emit_x)
    if wq is not None:
        pieces += _strassen(get_xn, *wq, emit_qkv)
    return st, r, pieces


def _layer(cfg, cur, nxt, o_s, xres, wo, wq, final_ref, consts, sbufs, mbufs, next_head, after_chunk):
    refs = tuple(x.bitcast(jnp.uint32) for x in cur) + (o_s,) + consts
    ou = o_s.bitcast(jnp.uint32)
    scores, softmax_pv = _attn_stages(cfg, *refs, 0, -10 ** 6)
    nstep = (DM // QC) * NG
    nd = S // DM
    tmax = nd * nstep - 1

    def body(c, _):
        _, _, pieces = _dense_pieces(c, xres, ou, wo, wq, nxt, final_ref)
        t0 = (c + 1) * nstep

        def step(s):
            scores(jnp.minimum(t0 + s + 1, tmax), sbufs[(s + 1) % 2], mbufs[(s + 1) % 2])
            softmax_pv(t0 + s, sbufs[s % 2], mbufs[s % 2])
        _interleave(pieces, [functools.partial(step, s) for s in range(nstep)], 1)
        after_chunk(c)
        return 0
    jax.lax.fori_loop(0, nd - 1, body, 0)
    _, _, pieces = _dense_pieces(nd - 1, xres, ou, wo, wq, nxt, final_ref)
    _interleave(pieces, next_head, 1)
    after_chunk(nd - 1)


def _kernel(x_hbm, aq_hbm, ao_hbm, bq_hbm, bo_hbm, out_hbm,
            xin, xres, aq, ao, bq, bo, aqs, aos, bqs, bos, q0, k0, v0, q1, k1, v1, o_s, s0, s1, m0, m1, bias, ones,
            sems, xsems, wsems):
    nd = S // DM
    npc = 3 * D // PN

    def rows(c):
        return pl.ds(pl.multiple_of(c * DM, DM), DM)

    def x_copy(c):
        return pltpu.make_async_copy(x_hbm.at[rows(c)], xin.at[rows(c)], xsems.at[c])

    def out_copy(c):
        return pltpu.make_async_copy(xin.at[rows(c)], out_hbm.at[rows(c)], xsems.at[c])

    aq_copies = [pltpu.make_async_copy(aq_hbm.at[:, pl.ds(n * PN, PN)], aq.at[:, pl.ds(n * PN, PN)],
                                       wsems.at[n]) for n in range(npc)]
    aq_order = [aq_copies[h * (npc // 2) + n] for n in range(npc // 2) for h in range(2)]
    cps = [pltpu.make_async_copy(src, dst, sems.at[i]) for i, (src, dst) in enumerate(
        [(ao_hbm, ao), (bq_hbm, bq), (bo_hbm, bo)])]
    x_copy(0).start()
    for c in aq_order:
        c.start()
    for c in range(1, nd):
        x_copy(c).start()
    for c in cps:
        c.start()

    d0 = jax.lax.broadcasted_iota(jnp.int32, (GR, 128), 0) - _lane_iota(GR) % KT
    for cfg in (CFG_A, CFG_B):
        for n, off in enumerate(cfg["offs"]):
            d = d0 + off
            ok = (d >= 0) & (d <= cfg["dmax"]) & (d % cfg["step"] == 0)
            bias[cfg["b0"] + n] = jnp.where(ok, 0.0, NEG).astype(jnp.float32)
    ri = jax.lax.broadcasted_iota(jnp.int32, (64, 128), 0)
    ones[...] = jnp.where((2 * ri) // DH == _lane_iota(64) // DH, jnp.uint32(0x3F803F80), jnp.uint32(0))

    buf0, buf1 = (q0, k0, v0), (q1, k1, v1)
    consts, sbufs, mbufs = (bias, ones), (s0, s1), (m0, m1)

    def head(cfg, cur):
        refs = tuple(x.bitcast(jnp.uint32) for x in cur) + (o_s,) + consts
        return _head_steps(cfg, refs, sbufs, mbufs)

    def first(c, steps=(), waits=None):
        x_copy(c).wait()
        st, r, pieces = _dense_pieces(c, xres, None, None, (aq, aqs), buf0, None)
        st["x0"] = xin[r, :].astype(jnp.float32)
        xres[r, :] = st["x0"]
        if waits is not None:
            def pre(n, p):
                waits[n].wait()
                waits[npc // 2 + n].wait()
                _prep_weights(aq, aqs, n)
                p()
            pieces = [functools.partial(pre, i // 3, p) if i % 3 == 0 else p for i, p in enumerate(pieces)]
        _interleave(pieces, steps, 0)

    first(0, waits=aq_copies)
    jax.lax.fori_loop(1, nd - 1, lambda c, _: first(c), None)
    first(nd - 1, head(CFG_A, buf0))

    def nothing(c):
        pass

    cps[0].wait()
    cps[1].wait()
    cps[2].wait()
    for w, ws in ((ao, aos), (bq, bqs), (bo, bos)):
        jax.lax.fori_loop(0, w.shape[1] // (2 * PN), lambda n, _: _prep_weights(w, ws, n), None)
    ao, bq, bo, aq = (ao, aos), (bq, bqs), (bo, bos), (aq, aqs)
    _layer(CFG_A, buf0, buf1, o_s, xres, ao, bq, None, consts, sbufs, mbufs, head(CFG_B, buf1), nothing)
    _layer(CFG_B, buf1, buf0, o_s, xres, bo, aq, None, consts, sbufs, mbufs, head(CFG_A, buf0), nothing)
    _layer(CFG_A, buf0, buf1, o_s, xres, ao, bq, None, consts, sbufs, mbufs, head(CFG_B, buf1), nothing)
    _layer(CFG_B, buf1, buf0, o_s, xres, bo, None, xin, consts, sbufs, mbufs, (),
           lambda c: out_copy(c).start())
    for c in range(nd):
        out_copy(c).wait()


@jax.jit
def pallas_interleave_layers__sliding_block__sliding_local_dilated__prompt_kernel(
    A_x: jax.Array,
    A_wqkv: jax.Array,
    A_wo: jax.Array,
    B_x: jax.Array,
    B_wqkv: jax.Array,
    B_wo: jax.Array,
):
    bf, f32 = jnp.bfloat16, jnp.float32
    NSLOT = len(_tiles(CFG_A, -10 ** 6)[1])
    out = pl.pallas_call(
        _kernel,
        out_shape=jax.ShapeDtypeStruct((S, D), bf),
        in_specs=[pl.BlockSpec(memory_space=pl.ANY)] * 5,
        out_specs=pl.BlockSpec(memory_space=pl.ANY),
        scratch_shapes=[
            pltpu.VMEM((S, D), bf), pltpu.VMEM((S, D), jnp.float32),
            pltpu.VMEM((D, 3 * D), bf), pltpu.VMEM((D, D), bf),
            pltpu.VMEM((D, 3 * D), bf), pltpu.VMEM((D, D), bf),
            *[pltpu.VMEM((5, D // 2, 3 * D // 2), bf), pltpu.VMEM((5, D // 2, D // 2), bf)] * 2,
            *[pltpu.VMEM((NG * GS, 128), bf) for _ in range(6)],
            pltpu.VMEM((NG * S, 128), bf),
            pltpu.VMEM((NSLOT, GR, 128), f32), pltpu.VMEM((NSLOT, GR, 128), f32),
            pltpu.VMEM((NU, GR, 128), f32), pltpu.VMEM((NU, GR, 128), f32),
            pltpu.VMEM((9, GR, 128), f32), pltpu.VMEM((64, 128), jnp.uint32),
            pltpu.SemaphoreType.DMA((3,)), pltpu.SemaphoreType.DMA((S // DM,)),
            pltpu.SemaphoreType.DMA((3 * D // PN,)),
        ],
        compiler_params=pltpu.CompilerParams(vmem_limit_bytes=110 * 2 ** 20),
    )(A_x.reshape(S, D), A_wqkv, A_wo, B_wqkv, B_wo)
    return out.reshape(1, S, D)
```
